```python
import os as _os
_os.environ.setdefault('JAX_PLATFORMS', 'cpu')
import jax
import jax.numpy as jnp

def _softmax(x, axis=-1):
    return jax.nn.softmax(x, axis=axis)

def _gelu(x):
    return jax.nn.gelu(x, approximate=True)

def _silu(x):
    return jax.nn.silu(x)

def _sigmoid(x):
    return jax.nn.sigmoid(x)

def _layernorm(x, axis=-1, eps=1e-05):
    m = jnp.mean(x, axis=axis, keepdims=True)
    v = jnp.var(x, axis=axis, keepdims=True)
    return (x - m) / jnp.sqrt(v + eps)

def _scatter_add(tgt, idx, src, axis=0):
    return tgt.at[idx].add(src)

def _segment_sum(src, seg, n):
    return jax.ops.segment_sum(src, seg, n)

class _Rng:

    def __init__(self, key):
        self._k = key

    def _next(self):
        self._k, sub = jax.random.split(self._k)
        return sub

    def normal(self, shape):
        return jax.random.normal(self._next(), shape, dtype=jnp.bfloat16)

    def randint(self, lo, hi, shape):
        return jax.random.randint(self._next(), shape, lo, hi, dtype=jnp.int32)

    def uniform(self, shape, lo=0.0, hi=1.0):
        return jax.random.uniform(self._next(), shape, jnp.bfloat16, lo, hi)

    def permutation(self, n):
        return jax.random.permutation(self._next(), n)
kernel_name = 'gated_mix__sliding_block__memory_aug_recurrent_mem_tr__prompt'

def setup_inputs():
    _rng = _Rng(jax.random.key(int.from_bytes(__import__("os").urandom(4), "little")))
    _w = lambda a: (lambda t: t.astype(jnp.bfloat16) if jnp.issubdtype(t.dtype, jnp.floating) else t)(jnp.asarray(a))

    def _A_setup():
        B, S, D = (1, 2048, 448)
        return {'x': _w((lambda *s: _rng.normal(s) * 0.05)(B, S, D)), 'wqkv': _w((lambda *s: _rng.normal(s) * 0.8)(D, 3 * D)), 'wo': _w((lambda *s: _rng.normal(s) * 0.05)(D, D))}
    _A_in = _A_setup()

    def _B_setup():
        B, S, Dm = (1, 2048, 448)
        H, Dh = (16, 256)
        M, seg = (8, 32)
        seg = min(seg, S)
        S = S // seg * seg
        return {'x': _w((lambda *s: _rng.normal(s) * 0.05)(B, S, Dm)), 'mem0': _w((lambda *s: _rng.normal(s) * 0.8)(B, M, Dm)), 'Wq': _w((lambda *s: _rng.normal(s) * 3.2)(Dm, H, Dh) * Dm ** (-0.5)), 'Wk': _w((lambda *s: _rng.normal(s) * 3.2)(Dm, H, Dh) * Dm ** (-0.5)), 'Wv': _w((lambda *s: _rng.normal(s) * 0.8)(Dm, H, Dh) * Dm ** (-0.5)), 'Wo': _w((lambda *s: _rng.normal(s) * 0.8)(H, Dh, Dm) * (H * Dh) ** (-0.5)), 'seg_len': seg}
    _B_in = _B_setup()
    return {'A_x': _A_in['x'], 'A_wqkv': _A_in['wqkv'], 'A_wo': _A_in['wo'], 'B_x': _B_in['x'], 'B_mem0': _B_in['mem0'], 'B_Wq': _B_in['Wq'], 'B_Wk': _B_in['Wk'], 'B_Wv': _B_in['Wv'], 'B_Wo': _B_in['Wo'], 'B_seg_len': _B_in['seg_len'], 'gate_w': _w((lambda *s: _rng.normal(s) * 0.05)(448) * 16.0)}

def reference(A_x, A_wqkv, A_wo, B_x, B_mem0, B_Wq, B_Wk, B_Wv, B_Wo, B_seg_len, gate_w):

    def _A_ref(x, wqkv, wo):
        B, S, D = x.shape
        H = 16
        Dh = D // H
        W = 256
        qkv = (lambda x, *d: x.transpose(*d))((x @ wqkv).reshape(B, S, 3, H, Dh), 2, 0, 3, 1, 4)
        q, k, v = (qkv[0], qkv[1], qkv[2])
        scores = jnp.einsum('bhqd,bhkd->bhqk', q, k) * Dh ** (-0.5)
        idx = jnp.arange(S)
        mask = (idx[:, None] - idx[None, :] >= 0) & (idx[:, None] - idx[None, :] < W)
        scores = jnp.where(mask[None, None], scores, -1000000000.0)
        p = _softmax(scores, axis=-1)
        o = jnp.einsum('bhqk,bhkd->bhqd', p, v)
        return (lambda x, *d: x.transpose(*d))(o, 0, 2, 1, 3).reshape(B, S, D) @ wo

    def _B_ref(x, mem0, Wq, Wk, Wv, Wo, seg_len):
        B, S, Dm = x.shape
        H, Dh = (Wq.shape[1], Wq.shape[2])
        M = mem0.shape[1]
        scale = Dh ** (-0.5)
        n_seg = S // seg_len
        L = M + seg_len
        idx = jnp.arange(L)
        mask = (idx[:, None] < M) | (idx[:, None] >= idx[None, :])
        mem = mem0
        outs = []
        for s in range(n_seg):
            xs = x[:, s * seg_len:(s + 1) * seg_len, :].copy()
            h = jnp.concatenate([mem, xs], axis=1)
            q = jnp.einsum('btd,dhe->bhte', h, Wq)
            k = jnp.einsum('btd,dhe->bhte', h, Wk)
            v = jnp.einsum('btd,dhe->bhte', h, Wv)
            scores = jnp.einsum('bhqe,bhke->bhqk', q, k) * scale
            scores = jnp.where(mask[None, None], scores, -1000000000.0)
            p = _softmax(scores, axis=-1)
            o = jnp.einsum('bhqk,bhke->bhqe', p, v)
            o = jnp.einsum('bhte,hed->btd', o, Wo)
            mem = o[:, :M, :].copy()
            outs.append(o[:, M:, :])
        return jnp.concatenate(outs, axis=1)
    x = A_x
    g = _sigmoid((x * gate_w).sum(-1, keepdims=True))
    a = _A_ref(x, A_wqkv, A_wo)
    b = _B_ref(x, B_mem0, B_Wq, B_Wk, B_Wv, B_Wo, B_seg_len)
    return g * a + (1 - g) * b
```

```python
import functools
import math

import jax
import jax.numpy as jnp
import jax.experimental.pallas as pl
import jax.experimental.pallas.tpu as pltpu

F32 = jnp.float32
BF16 = jnp.bfloat16
U32 = jnp.uint32
LOG2E = math.log2(math.e)
NEG = -1e30

NN = (((1,), (0,)), ((), ()))
NT = (((1,), (1,)), ((), ()))


def _dot(a, b, dims=NN):
    return jax.lax.dot_general(a, b, dims, preferred_element_type=F32)


def _iota(shape, dim):
    return jax.lax.broadcasted_iota(jnp.int32, shape, dim)


def _kernel(xT_hbm, wqkv_hbm, wo_hbm, mem0_ref, wq_hbm, wk_hbm, wv_hbm, woT_hbm, gw_ref,
            out_hbm,
            xT, wqkv, wo, wbuf, wBo, wqkvT, woT, xs, qT, kk, vT, gate, W, Zs, ZT, Ys, oT, bs, obuf,
            sem_x, sem_a, sem_w, sem_o):
    S, D = 2048, 448
    NB = S // 128
    XC = 4

    cp_wqkv = pltpu.make_async_copy(wqkv_hbm, wqkv, sem_a.at[0])
    cp_x = [pltpu.make_async_copy(xT_hbm.at[:, pl.ds(i * (S // XC), S // XC)],
                                  xT.at[:, pl.ds(i * (S // XC), S // XC)], sem_x.at[i])
            for i in range(XC)]
    cp_w = [[pltpu.make_async_copy(src.at[:, pl.ds(128 * c, 128)], wbuf.at[i, c], sem_w.at[2 * i + c])
             for c in range(2)] for i, src in enumerate((wq_hbm, wk_hbm, wv_hbm))]
    cp_wBo = pltpu.make_async_copy(woT_hbm, wBo, sem_w.at[6])
    cp_wo = pltpu.make_async_copy(wo_hbm, wo, sem_a.at[1])
    cp_wqkv.start()
    for cp in cp_x:
        cp.start()
    for i in range(3):
        for cp in cp_w[i]:
            cp.start()
    cp_wBo.start()
    cp_wo.start()

    lane = _iota((128, 128), 1)
    kpad = jnp.where(lane == 112, 1.0, 0.0).astype(BF16)
    for g in range(4):
        kk[g, 0:128, :] = kpad
        kk[g, 128:256, :] = kpad
    vT[0] = jnp.zeros((512, 128), BF16)
    vT[1] = jnp.zeros((512, 128), BF16)
    oT[...] = jnp.zeros(oT.shape, BF16)
    bs[...] = jnp.zeros(bs.shape, F32)

    cp_wqkv.wait()
    for j in range(10):
        wqkvT[128 * j:128 * (j + 1), :] = wqkv[:, 128 * j:128 * (j + 1)].T
    wqkvT[1280:1344, :] = wqkv[:, 1280:1344].T
    gw = jnp.broadcast_to(gw_ref[...].astype(F32), (8, D))
    qscale = 28 ** -0.5 * LOG2E

    def proj(b):
        xt = xT[:, pl.ds(pl.multiple_of(b * 128, 128), 128)]
        xe = jnp.concatenate([xt, xt[384:448]], axis=0)
        xs[pl.ds(pl.multiple_of(b * 128, 128), 128), :] = xe.T.astype(F32)
        gate[b] = jax.nn.sigmoid(_dot(gw, xt))
        sub = _iota((8, 128), 0)
        for g in range(4):
            q = _dot(wqkvT[112 * g:112 * (g + 1), :], xt)
            qT[b, 112 * g:112 * (g + 1), :] = (q * qscale).astype(BF16)
            k = _dot(wqkvT[D + 112 * g:D + 112 * (g + 1), :], xt)
            kt = jnp.concatenate([k.astype(BF16), jnp.zeros((16, 128), BF16)], axis=0)
            kk[g, pl.ds(pl.multiple_of(256 + b * 128, 128), 128), :] = kt.T
            v = _dot(wqkvT[2 * D + 112 * g:2 * D + 112 * (g + 1), :], xt)
            parts = []
            for i in range(2):
                r = 56 * i
                mid = v[r + 24:r + 32]
                parts += [v[r:r + 24], jnp.where(sub < 4, mid, 1.0),
                          jnp.where(sub < 4, 1.0, mid), v[r + 32:r + 56]]
            vT[b + 2, 128 * g:128 * (g + 1), :] = jnp.concatenate(parts, axis=0).astype(BF16)

    for i in range(XC):
        cp_x[i].wait()

        def proj_body(j, c, i=i):
            proj(i * (NB // XC) + 2 * j)
            proj(i * (NB // XC) + 2 * j + 1)
            return c
        jax.lax.fori_loop(0, NB // XC // 2, proj_body, 0)

    def load_pair(i, p):
        w = jnp.concatenate(
            [wbuf.at[i, c].bitcast(U32)[pl.ds(p, D, stride=8), :] for c in range(2)], axis=1)
        lo = pltpu.bitcast(w << 16, F32).astype(BF16)
        hi = pltpu.bitcast(w & jnp.uint32(0xFFFF0000), F32).astype(BF16)
        return lo, hi

    def fold(base, p, l0, l1, r0, r1, scale):
        tail = jnp.concatenate([r0[384:448], r1[384:448]], axis=0)
        half = _iota((D, 128), 1) < 64

        def put(n, val):
            if scale != 1.0:
                val = val * scale
            W[n] = pltpu.bitcast(val.astype(BF16), U32)
        o0 = _dot(l0, jnp.concatenate([r0[0:384], tail], axis=0), NT)
        o1 = _dot(l1, jnp.concatenate([r1[0:384], tail], axis=0), NT)
        put(base + p, jnp.where(half, o0[:, 384:512], o1[:, 384:512]))
        for c in range(3):
            put(base + 8 + 16 * c + 2 * p, o0[:, 128 * c:128 * (c + 1)])
            put(base + 8 + 16 * c + 2 * p + 1, o1[:, 128 * c:128 * (c + 1)])

    for cp in cp_w[0] + cp_w[1]:
        cp.wait()

    def foldA(p, c):
        q0, q1 = load_pair(0, p)
        k0, k1 = load_pair(1, p)
        fold(0, p, k0, k1, q0, q1, 256 ** -0.5 * LOG2E)
        return c
    for p in range(8):
        foldA(p, 0)

    for cp in cp_w[2]:
        cp.wait()
    cp_wBo.wait()

    def foldB(p, c):
        v0, v1 = load_pair(2, p)
        fold(56, p, v0, v1, wBo[2 * p], wBo[2 * p + 1], 1.0)
        return c
    for p in range(8):
        foldB(p, 0)

    cp_wo.wait()
    for j in range(3):
        woT[128 * j:128 * (j + 1), :] = wo[:, 128 * j:128 * (j + 1)].T
    woT[384:448, :] = wo[:, 384:448].T

    def wtile(n):
        return pltpu.bitcast(W[n], BF16)

    def pack_pair(dst, c, p, r0, r1):
        for t in range(5):
            dst[c, 128 * t + 16 * p:128 * t + 16 * p + 16, :] = jnp.concatenate(
                [r0[8 * t:8 * t + 8], r1[8 * t:8 * t + 8]], axis=0).astype(BF16)

    def big_pass(h, base, dst, c):
        for p in range(8):
            if c == 3:
                r = _dot(h, wtile(base + p))
                half = _iota((40, 128), 1) < 64
                pack_pair(dst, c, p, jnp.where(half, r, 0.0), jnp.where(half, 0.0, r))
            else:
                n = base + 8 + 16 * c + 2 * p
                pack_pair(dst, c, p, _dot(h, wtile(n)), _dot(h, wtile(n + 1)))

    def seg_allreduce(v, op):
        ln = _iota(v.shape, 1)
        for k in (1, 2, 4):
            v = op(v, jnp.where((ln & k) != 0, pltpu.roll(v, k, 1), pltpu.roll(v, 128 - k, 1)))
        return v

    def b_softmax(s):
        diag = (_iota((8, 128), 1) & 7) <= _iota((8, 128), 0)
        rows = []
        for a in range(5):
            ts = range(5) if a == 0 else range(a + 1)
            r = [s[8 * a:8 * a + 8, 128 * t:128 * (t + 1)] for t in ts]
            if a > 0:
                r[a] = jnp.where(diag, r[a], NEG)
            rows.append(r)
        m = jnp.concatenate([functools.reduce(jnp.maximum, r) for r in rows], axis=0)
        m = seg_allreduce(m, jnp.maximum)
        rows = [[jnp.exp2(x - m[8 * a:8 * a + 8]) for x in r] for a, r in enumerate(rows)]
        l = jnp.concatenate([functools.reduce(jnp.add, r) for r in rows], axis=0)
        inv = 1.0 / seg_allreduce(l, jnp.add)
        z = jnp.zeros((8, 128), F32)
        return jnp.concatenate(
            [jnp.concatenate([x * inv[8 * a:8 * a + 8] for x in r] + [z] * (5 - len(r)), axis=1)
             for a, r in enumerate(rows)], axis=0)

    def a_scores(qb, g):
        q = qT[qb, 112 * g:112 * (g + 1), :]
        row = _iota((112, 128), 0)
        bias = jnp.where(_iota((16, 128), 0) == 0, NEG, 0.0).astype(BF16)
        qs = [jnp.concatenate(
            [jnp.where((row >= 28 * i) & (row < 28 * (i + 1)), q, jnp.zeros_like(q)), bias], axis=0)
            for i in range(4)]
        k = kk[g, pl.ds(pl.multiple_of(qb * 128, 128), 384), :]
        return [_dot(k, qs[i]) for i in range(4)]

    def a_probs(st):
        upper = _iota((128, 128), 0) > _iota((128, 128), 1)
        e = jnp.where(upper, st[0:128], st[256:384])
        mid = st[128:256]
        mx = jnp.max(jnp.maximum(e, mid), axis=0, keepdims=True)
        pe = jnp.exp2(e - mx).astype(BF16)
        pm = jnp.exp2(mid - mx).astype(BF16)
        zero = jnp.zeros_like(pe)
        return jnp.concatenate([jnp.where(upper, pe, zero), pm, jnp.where(upper, zero, pe)], axis=0)

    def a_values(qb, g, ps, slot):
        sub = _iota((8, 128), 0)
        o = []
        for i in range(4):
            r = 128 * g + 32 * i
            v = jnp.concatenate([vT[qb + j, r:r + 32, :] for j in range(3)], axis=1)
            u = _dot(v, ps[i])
            l = u[28:29] if i % 2 == 0 else u[0:1]
            o.append(u * (1.0 / l))
        parts = []
        for i in (0, 2):
            parts += [o[i][0:24], jnp.where(sub < 4, o[i][24:32], o[i + 1][0:8]), o[i + 1][8:32]]
        oT[slot, 112 * g:112 * (g + 1), :] = jnp.concatenate(parts, axis=0).astype(BF16)

    def finish(qb, slot, g, bT):
        a = _dot(woT[112 * g:112 * (g + 1), :], oT[slot])
        gt = gate[qb][0:1]
        obuf[qb, 112 * g:112 * (g + 1), :] = (
            gt * a + (1.0 - gt) * bT[112 * g:112 * (g + 1)]).astype(BF16)

    def out_copy(qb):
        return pltpu.make_async_copy(
            obuf.at[qb], out_hbm.at[:, pl.ds(pl.multiple_of(qb * 128, 128), 128)], sem_o.at[qb])

    def step(qb, g, mem, bT):
        slot = qb % 2
        prev = jnp.maximum(qb - 1, 0)
        sts = a_scores(qb, g)
        finish(prev, 1 - slot, g, bT)
        x = xs[pl.ds(pl.multiple_of(qb * 128 + 32 * g, 32), 32), :]
        hf = jnp.concatenate([mem, x], axis=0)
        h = hf[:, 0:D]
        ps = [a_probs(st) for st in sts]
        for c in (3, 0, 1, 2):
            big_pass(h, 0, Zs, c)
            for t in range(5):
                ZT[t, 128 * c:128 * (c + 1), :] = Zs[c, 128 * t:128 * (t + 1), :].T
        a_values(qb, g, ps, slot)
        big_pass(h, 56, Ys, 3)
        s = jnp.concatenate([_dot(hf, ZT[t]) for t in range(5)], axis=1)
        big_pass(h, 56, Ys, 0)
        p = b_softmax(s)
        big_pass(h, 56, Ys, 1)
        o3 = _dot(p, Ys[3])
        o3 = o3 + pltpu.roll(o3, 64, 1)
        o0 = _dot(p, Ys[0])
        big_pass(h, 56, Ys, 2)
        o1 = _dot(p, Ys[1])
        o2 = _dot(p, Ys[2])
        o = jnp.concatenate([o0, o1, o2, o3], axis=1)
        bs[slot, 32 * g:32 * (g + 1), :] = o[8:40]
        return o[0:8]

    def main(qb, mem):
        bT = bs[1 - qb % 2].T
        for g in range(4):
            mem = step(qb, g, mem, bT)

        @pl.when(qb > 0)
        def _():
            out_copy(qb - 1).start()
        return mem

    m0 = mem0_ref[...].astype(F32)
    mem = jnp.concatenate([m0, m0[:, 384:448]], axis=1)
    jax.lax.fori_loop(0, NB, main, mem)

    bT = bs[(NB - 1) % 2].T
    for g in range(4):
        finish(NB - 1, (NB - 1) % 2, g, bT)
    out_copy(NB - 1).start()
    for qb in range(NB):
        out_copy(qb).wait()


@functools.partial(jax.jit, static_argnames=("B_seg_len",))
def pallas_gated_mix__sliding_block__memory_aug_recurrent_mem_tr__prompt_kernel(
    A_x, A_wqkv, A_wo, B_x, B_mem0, B_Wq, B_Wk, B_Wv, B_Wo, B_seg_len, gate_w,
):
    del B_x
    _, S, D = A_x.shape
    assert (S, D, B_seg_len) == (2048, 448, 32)
    xT = jnp.transpose(A_x.reshape(S, D))
    woT = jnp.transpose(B_Wo, (0, 2, 1))
    flat = lambda w: w.reshape(D * 16, 256)
    hbm = pl.BlockSpec(memory_space=pl.ANY)
    vmem = pl.BlockSpec(memory_space=pltpu.VMEM)
    NB = S // 128
    outT = pl.pallas_call(
        _kernel,
        out_shape=jax.ShapeDtypeStruct((D, S), BF16),
        in_specs=[hbm, hbm, hbm, vmem, hbm, hbm, hbm, hbm, vmem],
        out_specs=hbm,
        scratch_shapes=[
            pltpu.VMEM((D, S), BF16),
            pltpu.VMEM((D, 3 * D), BF16),
            pltpu.VMEM((D, D), BF16),
            pltpu.VMEM((3, 2, D * 16, 128), BF16),
            pltpu.VMEM((16, D, 256), BF16),
            pltpu.VMEM((3 * D, D), BF16),
            pltpu.VMEM((D, D), BF16),
            pltpu.VMEM((S, 512), F32),
            pltpu.VMEM((NB, D, 128), BF16),
            pltpu.VMEM((4, 256 + S, 128), BF16),
            pltpu.VMEM((NB + 2, 512, 128), BF16),
            pltpu.VMEM((NB, 8, 128), F32),
            pltpu.VMEM((112, D // 2, 128), U32),
            pltpu.VMEM((4, 640, 128), BF16),
            pltpu.VMEM((5, 512, 128), BF16),
            pltpu.VMEM((4, 640, 128), BF16),
            pltpu.VMEM((2, D, 128), BF16),
            pltpu.VMEM((2, 128, 512), F32),
            pltpu.VMEM((NB, D, 128), BF16),
            pltpu.SemaphoreType.DMA((4,)),
            pltpu.SemaphoreType.DMA((2,)),
            pltpu.SemaphoreType.DMA((7,)),
            pltpu.SemaphoreType.DMA((NB,)),
        ],
        compiler_params=pltpu.CompilerParams(vmem_limit_bytes=100 * 1024 * 1024),
    )(xT, A_wqkv, A_wo, B_mem0.reshape(8, D), flat(B_Wq), flat(B_Wk), flat(B_Wv), woT,
      gate_w.reshape(1, D))
    return jnp.transpose(outT).reshape(1, S, D)
```

```python
import functools
import math

import jax
import jax.numpy as jnp
import jax.experimental.pallas as pl
import jax.experimental.pallas.tpu as pltpu

F32 = jnp.float32
BF16 = jnp.bfloat16
U32 = jnp.uint32
LOG2E = math.log2(math.e)
NEG = -1e30

S, D = 2048, 448
NB = S // 128
XC = 4
PER = NB // XC

NN = (((1,), (0,)), ((), ()))
NT = (((1,), (1,)), ((), ()))


def _dot(a, b, dims=NN):
    return jax.lax.dot_general(a, b, dims, preferred_element_type=F32)


def _iota(shape, dim):
    return jax.lax.broadcasted_iota(jnp.int32, shape, dim)


def _tile(i):
    return slice(128 * i, 128 * (i + 1))


_HK = (
    ((0, 0, 0, 0, -1, 0), (0, 0, 0, -1, 1, 0, 1, 0, 0), (1, 0, 0, 1, 0, 0)),
    ((1, -1, 0, -1, 1, 0), (1, 0, 0, 0, 0, 0, 0, 0, 0), (0, 0, 0, -1, -1, 0)),
    ((0, 0, 1, 0, 1, 0), (0, 0, 0, 0, 0, -1, 1, 0, 0), (1, 0, 0, 0, 0, -1)),
    ((1, -1, 0, 0, 0, 0), (0, 0, 0, 0, 1, 0, 0, 0, 0), (-1, -1, 0, -1, -1, 0)),
    ((0, 0, 0, 0, -1, -1), (0, 0, 0, 0, 0, 0, -1, 0, 0), (0, 0, 0, 1, 0, 1)),
    ((0, 0, 1, -1, 0, -1), (0, 0, -1, 0, 0, 0, 0, -1, 0), (0, -1, 1, 0, 0, 1)),
    ((-1, 1, 0, 0, -1, 0), (1, 0, 0, 0, 1, 0, 0, 0, 0), (-1, 0, 0, -1, -1, 0)),
    ((0, 0, 1, 0, 0, -1), (0, 0, 1, 0, 0, 0, 1, 0, -1), (0, 0, 0, 0, 0, 1)),
    ((0, 0, 1, 0, 0, 0), (0, 0, 0, 0, 0, -1, 0, 1, 1), (0, 0, 1, 0, 0, 1)),
    ((0, 0, 0, 1, 0, 1), (0, 0, 0, 0, 0, 0, 0, -1, 0), (0, -1, 1, 0, -1, 1)),
    ((1, 0, 0, 0, 0, 0), (0, 1, 1, 0, 1, 0, 0, 0, 0), (0, 1, 0, 0, 0, 0)),
    ((0, -1, 0, 0, 1, 0), (-1, 0, 0, -1, 0, 1, 0, 0, 0), (1, 0, 0, 0, 0, 0)),
    ((0, 0, 0, 1, 0, 0), (1, -1, 0, 0, 0, 0, 0, 1, 0), (0, 0, 0, 0, -1, 0)),
    ((-1, 0, -1, 1, 0, 1), (0, 0, 1, 0, 0, 0, 0, 0, 0), (0, 1, -1, 0, 0, 0)),
    ((0, 1, 1, 0, 0, 0), (0, 0, 0, 0, 0, 1, 0, 0, 0), (1, 0, 1, 0, 0, 0)),
)
_HALVES = (
    ((7, 1, (0, 0, -1), (0, 0, 1)), (4, 1, (0, -1, -1), (1, 0, 1)), (2, 1, (0, -1, 0), (0, 0, 1)),
     (5, 1, (-1, 0, -1), (0, 0, 1)), (0, 1, (0, -1, 0), (1, 0, 0)), (3, 1, (0, 1, 0), (1, 1, 0)),
     (1, 1, (1, 0, 0), (1, 1, 0)), (12, 1, (-1, 0, 0), (0, 1, 0)), (9, 0, (-1, 0, -1), (0, 1, -1))),
    ((11, 1, (0, -1, 0), (1, 0, 0)), (14, 1, (0, 1, 1), (1, 0, 1)), (8, 1, (0, 0, 1), (0, 0, 1)),
     (9, 1, (0, 0, -1), (0, 1, -1)), (13, 1, (-1, 0, 0), (0, 1, -1)), (6, 1, (-1, 1, 0), (0, 1, 0)),
     (10, 1, (1, 0, 0), (0, 1, 0)), (2, 0, (0, 0, 1), (1, 0, 0)), (1, 0, (1, -1, 0), (1, 1, 0))),
)


def _triples():
    out, loose = [], []
    for kind in "zy":
        for p in range(8):
            out += [[(kind, c, p, h) for c in range(3)] for h in range(2)]
            for tile in ([("t", 0, p, 0)] if kind == "z" else []) + [(kind, 3, p, 0)]:
                loose.append(tile)
                if len(loose) == 3:
                    out.append(loose)
                    loose = []
    return out


_TRIPLES = _triples()
_LOOSE = [n for n, t in enumerate(_TRIPLES) if t[2][1] != 2]
_MIXED = [n for n, t in enumerate(_TRIPLES) if t[0][0] != "y" and t[2][0] == "y"]
_ISSUE = ([n for n, t in enumerate(_TRIPLES) if t[0][0] != "y"]
          + [n for n, t in enumerate(_TRIPLES) if t[0][0] == "y"][::-1])


def _half(n, first):
    return _HALVES[int((_ISSUE.index(n) < len(_ISSUE) // 2) != first)]


def _combine(coefs, vals):
    terms = sorted(((c, j) for j, c in enumerate(coefs) if c), key=lambda t: (-t[0], t[1]))
    out = vals[terms[0][1]] if terms[0][0] > 0 else -vals[terms[0][1]]
    for c, j in terms[1:]:
        out = out + vals[j] if c > 0 else out - vals[j]
    return out


class _Sums:
    def __init__(self, coefs):
        self.coefs = coefs
        self.left = [sum(c[o] != 0 for c in coefs) for o in range(len(coefs[0]))]
        self.acc = {}

    def add(self, k, v):
        done = []
        for o, c in enumerate(self.coefs[k]):
            if not c:
                continue
            if o not in self.acc:
                self.acc[o] = (c, v)
            else:
                sign, a = self.acc[o]
                if sign == c:
                    self.acc[o] = (sign, a + v)
                else:
                    self.acc[o] = (1, a - v if sign > 0 else v - a)
            self.left[o] -= 1
            if not self.left[o]:
                done.append((o,) + self.acc[o])
        return done


def _schedule(first):
    jobs = [("w", ([n], k)) for n in _ISSUE for k, j in enumerate(_half(n, first)) if j[1]]
    woven, end, at8, at7 = _ORDER[first]
    short = {}
    for i in range(0, len(_ISSUE), 4):
        ns = _ISSUE[i:i + 4]
        row = jobs.index(("w", (ns[:1], 0))) // 4
        has7 = _half(ns[0], first)[7][1]
        short.setdefault(row + at8[has7], []).append(("w", (ns, 8)))
        if not has7:
            short.setdefault(row + at7, []).append(("w", (ns, 7)))
    plan = []
    for row in range(len(jobs) // 4):
        plan += short.get(row, []) + woven.get(row, []) + jobs[4 * row:4 * row + 4]
    return plan + end


_ORDER = {
    True: (
        {0: [("cor", 0)], 4: [("s1", 1)], 12: [("tq", 0), ("s1", 4)], 20: [("tq", 1), ("s1", 3)],
         29: [("head", 0), ("s1", 2)], 37: [("head", 1)],
         47: [("s2", 0), ("s1", 0), ("softmax", 0)], 53: [("head", 2)], 60: [("head", 3)]},
        [("tv", 0), ("av", 0), ("y", 4), ("y", 1), ("u", 0), ("y", 3), ("u", 1), ("y", 2),
         ("y", 0), ("u", 2), ("u", 4), ("u", 3), ("u", 5), ("u", 6), ("u", 7), ("fin", 0)],
        (1, 1), 3),
    False: (
        {2: [("cor", 0), ("tq", 0)], 6: [("tq", 1)], 15: [("head", 0)],
         41: [("s2", 0), ("s1", 0)], 46: [("head", 1)], 47: [("s1", 4)], 50: [("s1", 1)],
         53: [("head", 2)], 54: [("s1", 3)], 58: [("s1", 2), ("softmax", 0)], 63: [("head", 3)]},
        [("av", 0), ("y", 1), ("y", 4), ("y", 0), ("tv", 0), ("y", 3), ("u", 2), ("y", 2),
         ("u", 0), ("u", 1), ("u", 3), ("u", 4), ("u", 6), ("u", 5), ("u", 7), ("fin", 0)],
        (1, 1), 4),
}


def _kernel(xT_hbm, wqkv_hbm, wo_hbm, mem0_hbm, wq_hbm, wk_hbm, wv_hbm, woT_hbm, gw_hbm,
            out_hbm,
            xT, wqkv, wo, wbuf, wBo, wqkvT, woT, xs, qT, kk, k2, vT, gate, W, WT, WU, heads,
            Zs, Ys, part, Ts, Tq, scales, raw, oT, oP, bs, bT, obuf, tri, mem0, gw,
            sem_x, sem_a, sem_w, sem_o):
    cp_x = [pltpu.make_async_copy(xT_hbm.at[:, pl.ds(i * (S // XC), S // XC)], xT.at[i], sem_x.at[i])
            for i in range(XC)]
    cp_wqkv = [pltpu.make_async_copy(wqkv_hbm.at[:, cols], wqkv.at[:, cols], sem_a.at[i])
               for i, cols in enumerate((pl.ds(0, 512), pl.ds(512, 3 * D - 512)))]
    cp_mem = pltpu.make_async_copy(mem0_hbm, mem0, sem_a.at[2])
    cp_gw = pltpu.make_async_copy(gw_hbm, gw, sem_a.at[3])
    cp_wo = pltpu.make_async_copy(wo_hbm, wo, sem_a.at[4])
    cp_w = [[pltpu.make_async_copy(src.at[:, pl.ds(128 * c, 128)], wbuf.at[i, c], sem_w.at[2 * i + c])
             for c in range(2)] for i, src in enumerate((wq_hbm, wk_hbm, wv_hbm))]
    cp_wBo = pltpu.make_async_copy(woT_hbm, wBo, sem_w.at[6])
    cp_wqkv[0].start()
    cp_x[0].start()

    kpad = jnp.where(_iota((128, 128), 1) == 112, 1.0, 0.0).astype(BF16)
    for j in range(2):
        for g in range(4):
            kk[g, _tile(j), :] = kpad
        vT[j] = jnp.zeros((512, 128), BF16)
    r2, col = 2 * _iota((64, 128), 0), _iota((64, 128), 1)
    tri[...] = (jnp.where(r2 > col, jnp.uint32(0xFFFF), 0)
                | jnp.where(r2 + 1 > col, jnp.uint32(0xFFFF0000), 0)).astype(U32)
    oT[...] = jnp.zeros(oT.shape, BF16)
    bs[...] = jnp.zeros(bs.shape, BF16)

    def q_proj(i, j):
        xt = xT[i, :, _tile(j)]
        for g in range(4):
            q = _dot(wqkvT[112 * g:112 * (g + 1), :], xt)
            qT[i * PER + j, 112 * g:112 * (g + 1), :] = (q * (28 ** -0.5 * LOG2E)).astype(BF16)

    def kv_proj(i):
        for j in range(PER):
            b = i * PER + j
            xt = xT[i, :, _tile(j)]
            for g in range(4):
                k = _dot(wqkvT[D + 112 * g:D + 112 * (g + 1), :], xt)
                kn = jnp.concatenate([k.astype(BF16), jnp.zeros((16, 128), BF16)], axis=0).T
                kk[g, pl.ds(pl.multiple_of(256 + b * 128, 128), 128), :] = kn
                khi = pltpu.bitcast(kn[32:128], U32)
                k2[g, b] = pltpu.bitcast(jnp.where(_iota((48, 128), 1) < 56, pltpu.roll(khi, 72, 1),
                                                   pltpu.roll(khi, 56, 1)), BF16)
        sub = _iota((8, 128), 0)
        for j in range(PER):
            b = i * PER + j
            xt = xT[i, :, _tile(j)]
            xs[pl.ds(pl.multiple_of(b * 128, 128), 128), :] = jnp.concatenate([xt, xt[384:D]], axis=0).T
            for g in range(4):
                v = _dot(wqkvT[2 * D + 112 * g:2 * D + 112 * (g + 1) + (16 if g == 3 else 0), :], xt)
                if g == 3:
                    gate[b] = jax.nn.sigmoid(v[112:120])
                parts = []
                for r in (0, 56):
                    mid = v[r + 24:r + 32]
                    parts += [v[r:r + 24], jnp.where(sub < 4, mid, 1.0),
                              jnp.where(sub < 4, 1.0, mid), v[r + 32:r + 56]]
                vT[b + 2, _tile(g), :] = jnp.concatenate(parts, axis=0).astype(BF16)

    cp_wqkv[0].wait()
    for cp in (cp_x[1], cp_wqkv[1], cp_gw, cp_mem):
        cp.start()
    for j in range(4):
        wqkvT[_tile(j), :] = wqkv[:, _tile(j)].T
    cp_x[0].wait()
    for j in range(PER):
        q_proj(0, j)
    for cp in (cp_x[1], cp_wqkv[1], cp_gw, cp_mem):
        cp.wait()
    for cp in cp_x[2:] + cp_w[0] + cp_w[1]:
        cp.start()
    m0 = mem0[...].astype(F32)
    m0 = jnp.concatenate([m0, m0[:, 384:D]], axis=1)
    wqkvT[3 * D:3 * D + 16, :] = jnp.broadcast_to(gw[...].astype(F32).reshape(1, D), (16, D)).astype(BF16)
    for j in range(4, 11):
        cols = slice(128 * j, min(128 * (j + 1), 3 * D))
        wqkvT[cols, :] = wqkv[:, cols].T
    for j in range(PER):
        q_proj(1, j)

    def kv_body(i, c):
        @pl.when(i == 1)
        def _():
            for cp in cp_x[2:]:
                cp.wait()
            for cp in cp_w[2]:
                cp.start()
        kv_proj(2 * i)
        kv_proj(2 * i + 1)
        return c
    jax.lax.fori_loop(0, XC // 2, kv_body, 0)

    def token_operands(x):
        blocks = [x[32 * i:32 * (i + 1), _tile(k)] for i in range(2) for k in range(3)]
        return [_combine(u, blocks) for u, _, _ in _HK]

    stored = {}

    def tokens(n, k, first, r, sums):
        if n not in sums:
            coefs = [[c * j[1] for c in _HK[j[0]][2]] for j in _half(n, first)]
            if not first:
                coefs += [[stored[n, o] * (o == q) for o in range(6)] for q in range(6)]
            sums[n] = _Sums(coefs)
        if first:
            for o, sign, v in sums[n].add(k, r):
                part[n, o] = v
                stored[n, o] = sign
            return []
        for o, c in enumerate(sums[n].coefs[k]):
            if c and o not in sums[n].acc:
                sums[n].add(9 + o, part[n, o])
        return sums[n].add(k, r)

    tok0 = token_operands(xs[0:64, 0:384].astype(F32))
    loose, ready, fresh, late, leftover = [0], [], [], [], []

    def put_triple(n, slots):
        blocks = [raw[slots[j], _tile(k), :] for k in range(3) for j in range(3)]
        for i, (_, v, _) in enumerate(_HK):
            W[n, i] = pltpu.bitcast(_combine(v, blocks).astype(BF16), U32)
        (late if n in _MIXED else fresh).append(n)

    def put_loose(tile):
        at, j = divmod(loose[0], 3)
        if _LOOSE[at] in _MIXED:
            m = functools.reduce(jnp.maximum, [jnp.abs(v) for v in tile])
            m = jnp.max(jnp.max(m, axis=0, keepdims=True), axis=1, keepdims=True)
            m = jnp.clip(jnp.broadcast_to(m, (8, 128)), 2.0 ** -60, 2.0 ** 60)
            bits = pltpu.bitcast(m, U32) & jnp.uint32(0x7F800000)
            scales[j] = pltpu.bitcast(bits, F32)
            tile = [v * pltpu.bitcast(jnp.uint32(0x7F000000) - bits, F32)[0:1] for v in tile]
        for k in range(3):
            raw[6 + loose[0] % 6, _tile(k), :] = tile[k]
        loose[0] += 1
        if j == 2:
            ready.append(at)

    def put_ready():
        while ready:
            at = ready.pop(0)
            put_triple(_LOOSE[at], [6 + (3 * at + j) % 6 for j in range(3)])

    def warm_up(count):
        for _ in range(min(count, len(fresh))):
            n, sums = fresh.pop(0), {}
            for k, j in enumerate(_half(n, True)):
                if j[1]:
                    tokens(n, k, True, _dot(tok0[j[0]], pltpu.bitcast(W[n, j[0]], BF16)), sums)

    def unpack(i, p):
        for c in range(2):
            w = wbuf.at[i, c].bitcast(U32)[pl.ds(p, D, stride=8), :]
            lo = pltpu.bitcast(w << 16, F32).astype(BF16)
            hi = pltpu.bitcast(w & jnp.uint32(0xFFFF0000), F32).astype(BF16)
            heads[p % 2, i % 2, 0, c] = pltpu.bitcast(lo, U32)
            heads[p % 2, i % 2, 1, c] = pltpu.bitcast(hi, U32)

    def unpacked(i, p, h):
        return lambda lo, hi: jnp.concatenate(
            [pltpu.bitcast(heads[p % 2, i % 2, h, c, lo // 2:hi // 2, :], BF16) for c in range(2)], axis=1)

    def fold(kind, p, left, right, prefetch):
        cols, rows = [], []
        for c in range(3):
            for h, j in (divmod(2 * c, 3), divmod(2 * c + 1, 3)):
                v = _dot(left[h](0, D), right[h](128 * j, 128 * (j + 1)), NT)
                raw[3 * h + j] = v[0:384]
                rows.append(v[384:D])
            cols.append(jnp.concatenate(
                [_dot(right[h](384, D), left[h](128 * c, 128 * (c + 1)), NT) for h in range(2)], axis=0).T)
            warm_up(2 if c == 1 else 1)
            prefetch(c)
            if c == 0:
                a, b = (right, left) if kind == "z" else (left, right)
                both = jnp.concatenate([b[h](384, D) for h in range(2)], axis=0)
                corner = [_dot(a[h](384, D), both, NT) for h in range(2)]
                put_ready()
                while leftover:
                    put_loose(leftover.pop(0))
            else:
                put_triple(_TRIPLES.index([(kind, j, p, c - 1) for j in range(3)]), range(3 * c - 3, 3 * c))
        return cols, [jnp.concatenate([rows[c], rows[3 + c]], axis=0) for c in range(3)], corner

    for cp in cp_w[0] + cp_w[1]:
        cp.wait()
    cp_wBo.start()
    cp_wo.start()
    unpack(0, 0)
    unpack(1, 0)
    q_proj(2, 0)
    q_proj(2, 1)
    half = _iota((64, 128), 1) < 64
    for p in range(8):
        def prefetch(c):
            if p < 7 and c < 2:
                unpack(c, p + 1)
        cols, rows, corner = fold("z", p, [unpacked(1, p, h) for h in range(2)],
                                  [unpacked(0, p, h) for h in range(2)], prefetch)
        leftover += [[v.T for v in rows], cols]
        WT[p] = pltpu.bitcast(jnp.where(half, *corner).astype(BF16), U32)
    q_proj(2, 2)
    q_proj(2, 3)
    for cp in cp_w[2] + [cp_wBo, cp_wo]:
        cp.wait()
    unpack(2, 0)
    q_proj(3, 0)
    q_proj(3, 1)
    for p in range(8):
        def prefetch(c):
            if p < 7 and c == 0:
                unpack(2, p + 1)
            if p < 4 and c == 1:
                span = slice(128 * p, min(128 * (p + 1), D))
                woT[span, :] = wo[:, span].T
        cols, rows, corner = fold("y", p, [unpacked(2, p, h) for h in range(2)],
                                  [lambda lo, hi, h=h: wBo[2 * p + h, lo:hi, :] for h in range(2)], prefetch)
        leftover.append(cols)
        rows.append(jnp.concatenate([jnp.where(half, corner[0], 0.0), jnp.where(half, 0.0, corner[1])], axis=0))
        for c in range(4):
            WU[p, c] = pltpu.bitcast(rows[c].astype(BF16), U32)
    put_loose(leftover.pop())
    fresh += late
    q_proj(3, 2)
    warm_up(len(fresh))
    put_ready()
    q_proj(3, 3)
    warm_up(len(fresh))

    def emit(n, j, t0, sign, v, st):
        kind, c, p, h = _TRIPLES[n][j]
        v = v if sign > 0 else -v
        if n in _MIXED:
            v = v * jnp.concatenate([scales[j]] * (v.shape[0] // 8), axis=0)
        if kind == "t":
            if t0 == 5:
                Ts[p] = v
            else:
                st["t", p, t0] = v
            return
        if c == 3:
            left = _iota(v.shape, 1) < 64
            pair = [jnp.where(left, v, 0.0), jnp.where(left, 0.0, v)]
        else:
            st[kind, c, p, h, t0] = v
            if (kind, c, p, 1 - h, t0) not in st:
                return
            pair = [st[kind, c, p, i, t0] for i in range(2)]
        for t in range(v.shape[0] // 8):
            (Zs if kind == "z" else Ys)[t0 + t, c, 16 * p:16 * p + 16, :] = jnp.concatenate(
                [u[8 * t:8 * t + 8] for u in pair], axis=0).astype(BF16)

    def project(ns, k, first, tok, mem, st):
        i, has_tok, a, _ = _half(ns[0], first)[k]
        rows = [_combine(a, [mem[:, _tile(j)] for j in range(3)])] + ([tok[i]] if has_tok else [])
        r = _dot(jnp.concatenate(rows, axis=0),
                 jnp.concatenate([pltpu.bitcast(W[n, i], BF16) for n in ns], axis=1))
        for j, n in enumerate(ns):
            sums = st["mem"].setdefault(n, _Sums([q[3] for q in _half(n, first)]))
            for o, sign, v in sums.add(k, r[0:8, _tile(j)]):
                emit(n, o, 0, sign, v, st)
            if has_tok:
                for o, sign, v in tokens(n, k, first, r[8:40], st["tok"]):
                    emit(n, o % 3, 1 + 4 * (o // 3), sign, v, st)

    def key_tile(src, first, t):
        i = t + 4 * first if t else 0
        return jnp.concatenate([src[i, c] for c in range(4)], axis=1)

    def rows_of(t):
        return [0] + list(range(max(t, 1), 5))

    def take(v, groups):
        return jnp.concatenate([v[8 * a:8 * a + 8] for a in groups], axis=0)

    def spread(v, groups):
        return {a: v[8 * n:8 * n + 8] for n, a in enumerate(groups)}

    def tail_rows(hf):
        left = _iota((8, 128), 1) < 64
        return [jnp.concatenate([jnp.where(left, hf[8 * t:8 * t + 8, 384:512], 0.0),
                                 jnp.where(left, 0.0, hf[8 * t:8 * t + 8, 384:512])], axis=0).astype(BF16)
                for t in range(5)]

    def pick(srcs, bit=4):
        if len(srcs) == 1:
            return next(iter(srcs.values()))
        lo = {q: v for q, v in srcs.items() if not q & bit}
        hi = {q: v for q, v in srcs.items() if q & bit}
        if not lo or not hi:
            return pick(srcs, bit // 2)
        return jnp.where((_iota((8, 128), 1) & (16 * bit)) != 0, pick(hi, bit // 2), pick(lo, bit // 2))

    def tail_scores(tq, vr):
        vm = jnp.concatenate(vr + [jnp.zeros((48, 128), BF16)], axis=0)
        o = []
        for q in range(4):
            r = _dot(jnp.concatenate(tq[2 * q:2 * q + 2], axis=0), vm, NT)
            o += [r[0:40], r[40:80]]
        o = [pltpu.roll(v, 16 * p, 1) if p else v for p, v in enumerate(o)]
        out = []
        for t in range(5):
            r = jnp.concatenate(
                [pick({(p + t) % 8: o[p][8 * a:8 * a + 8] for p in range(8)}) for a in rows_of(t)], axis=0)
            out.append(spread(pltpu.roll(r, 128 - 16 * t, 1) if t else r, rows_of(t)))
        return out

    def tail_values(pr, vr):
        q = [spread(pltpu.roll(pr[t], 16 * t, 1) if t else pr[t], rows_of(t)) for t in range(5)]
        z32, z16 = jnp.zeros((8, 128), F32), jnp.zeros((16, 128), BF16)
        u = []
        for p in range(8):
            l = jnp.concatenate(
                [pick({(p + t) % 8: q[t].get(a, z32) for t in range(5)}) for a in range(5)], axis=0)
            vm = jnp.concatenate([vr[(j - p) % 8] if (j - p) % 8 < 5 else z16 for j in range(8)], axis=0)
            u.append(_dot(l, vm))
        return u

    def seg_allreduce(v, op):
        ln = _iota(v.shape, 1) & 7
        r = [v] + [jnp.where(ln >= k, pltpu.roll(v, k, 1), pltpu.roll(v, 120 + k, 1)) for k in range(1, 8)]
        return op(op(op(r[0], r[1]), op(r[2], r[3])), op(op(r[4], r[5]), op(r[6], r[7])))

    def b_softmax(s1, s2):
        diag = (_iota((8, 128), 1) & 7) <= _iota((8, 128), 0)
        rows = [{t: (s1[t][a] + s2[t][a]) * (256 ** -0.5 * LOG2E) for t in range(5) if a in s1[t]}
                for a in range(5)]
        for a in range(1, 5):
            rows[a][a] = jnp.where(diag, rows[a][a], NEG)
        m = jnp.concatenate([functools.reduce(jnp.maximum, r.values()) for r in rows], axis=0)
        m = seg_allreduce(m, jnp.maximum)
        rows = [{t: jnp.exp2(x - m[8 * a:8 * a + 8]) for t, x in r.items()} for a, r in enumerate(rows)]
        l = jnp.concatenate([functools.reduce(jnp.add, r.values()) for r in rows], axis=0)
        inv = 1.0 / seg_allreduce(l, jnp.add)
        return [jnp.concatenate([rows[a][t] * inv[8 * a:8 * a + 8] for a in rows_of(t)], axis=0)
                for t in range(5)]

    def head_only(q32, i):
        lo, hi = 14 * i // 8 * 8, -(-14 * (i + 1) // 8) * 8
        row = _iota((hi - lo, 128), 0) + lo
        kept = jnp.where((row >= 14 * i) & (row < 14 * (i + 1)), q32[lo:hi], 0)
        parts = [jnp.zeros((lo, 128), U32), kept, jnp.zeros((56 - hi, 128), U32)]
        return jnp.concatenate([v for v in parts if v.shape[0]], axis=0)

    def a_corners(qb, g, i):
        q = pltpu.bitcast(qT[qb, 112 * g:112 * (g + 1), :], U32)
        own = head_only(q, i)
        swapped = head_only(jnp.concatenate([q[28:56], q[0:28]], axis=0), (i + 2) % 4)
        old = pltpu.bitcast(kk[g, pl.ds(pl.multiple_of(qb * 128, 128), 96), :], U32)
        new = pltpu.bitcast(k2[g, qb], U32)
        ln = _iota((48, 128), 1)
        keys = pltpu.bitcast(jnp.where(((ln >= 56) & (ln < 112)) if i < 2 else (ln < 56), new, old), BF16)
        out = []
        for r in range(3):
            cut = 32 * (r + 1)
            qs = pltpu.bitcast(jnp.where(_iota((56, 128), 1) < cut, own, swapped), BF16)
            bias = jnp.where((_iota((16, 128), 0) == 0) & (_iota((16, 128), 1) < cut), NEG, 0.0)
            out.append(_dot(keys[32 * r:32 * r + 32], jnp.concatenate([qs, bias.astype(BF16)], axis=0)))
        return out

    def a_probs(qb, g, i, corner):
        q = pltpu.bitcast(qT[qb, 112 * g:112 * (g + 1), :], U32)
        bias = jnp.where(_iota((16, 128), 0) == 0, NEG, 0.0).astype(BF16)
        qs = jnp.concatenate([pltpu.bitcast(head_only(q, i), BF16), bias], axis=0)
        sc = jnp.concatenate(
            [_dot(kk[g, pl.ds(pl.multiple_of(qb * 128 + 96 + 48 * j, 16), 48), :], qs) for j in range(4)], axis=0)
        upper = _iota((128, 128), 0) > _iota((128, 128), 1)
        edge = jnp.where(upper, jnp.concatenate(corner + [sc[0:32]], axis=0),
                         jnp.concatenate([sc[160:192]] + corner, axis=0))
        mid = sc[32:160]
        mx = jnp.max(jnp.maximum(edge, mid), axis=0, keepdims=True)
        pe = pltpu.bitcast(jnp.exp2(edge - mx).astype(BF16), U32)
        pm = jnp.exp2(mid - mx).astype(BF16)
        older = pe & tri[...]
        return jnp.concatenate([pltpu.bitcast(older, BF16), pm, pltpu.bitcast(pe ^ older, BF16)], axis=0)

    def a_values(qb, g, ps):
        sub = _iota((8, 128), 0)
        o = []
        for i in range(4):
            r = 128 * g + 32 * i
            u = _dot(jnp.concatenate([vT[qb + j, r:r + 32, :] for j in range(3)], axis=1), ps[i])
            o.append(u * (1.0 / (u[28:29] if i % 2 == 0 else u[0:1])))
        parts = []
        for i in (0, 2):
            parts += [o[i][0:24], jnp.where(sub < 4, o[i][24:32], o[i + 1][0:8]), o[i + 1][8:32]]
        oT[112 * g:112 * (g + 1), :] = jnp.concatenate(parts, axis=0).astype(BF16)

    def retire():
        oP[...] = oT[...]
        bT[...] = bs[...].T

    def finish(qb, g):
        rows = slice(112 * g, 112 * (g + 1))
        a = _dot(woT[rows, :], oP[...])
        gt = gate[qb][0:1]
        obuf[qb, rows, :] = (gt * a + (1.0 - gt) * bT[rows, :].astype(F32)).astype(BF16)

    def out_copy(qb):
        return pltpu.make_async_copy(
            obuf.at[qb], out_hbm.at[:, pl.ds(pl.multiple_of(qb * 128, 128), 128)], sem_o.at[qb])

    def step(qb, g, mem):
        x = xs[pl.ds(pl.multiple_of(qb * 128 + 32 * g, 32), 32), :]
        hf = jnp.concatenate([mem, x.astype(F32)], axis=0)
        first = g % 2 == 1
        start = qb * 128 + 64 * ((g + 1) // 2)
        if g == 3:
            start = jnp.minimum(start, S - 64)
        tok = token_operands(xs[pl.ds(pl.multiple_of(start, 64), 64), 0:384].astype(F32))
        vr = tail_rows(hf)
        st, s1, ps, acc = dict(mem={}, tok={}), {}, [], {}

        def add(r):
            for a, v in r.items():
                acc[a] = acc[a] + v if a in acc else v
        for kind, i in _schedule(first):
            if kind == "w":
                project(*i, first, tok, mem, st)
            elif kind == "tq":
                for p in range(4 * i, 4 * i + 4):
                    Tq[p] = _dot(hf[:, 384:D], pltpu.bitcast(WT[p], BF16))
            elif kind == "s2":
                s2 = tail_scores(
                    [Tq[p] + jnp.concatenate([st["t", p, 0], Ts[p] if first else st["t", p, 1]], axis=0)
                     for p in range(8)], vr)
            elif kind == "s1":
                s1[i] = spread(_dot(take(hf, rows_of(i)), key_tile(Zs, first, i), NT), rows_of(i))
            elif kind == "softmax":
                pr = b_softmax(s1, s2)
            elif kind == "tv":
                u = tail_values(pr, vr)
            elif kind == "y":
                add(spread(_dot(pr[i], key_tile(Ys, first, i)), rows_of(i)))
            elif kind == "u":
                w = jnp.concatenate([pltpu.bitcast(WU[i, c], BF16) for c in range(4)], axis=1)
                add(spread(_dot(u[i], w), range(5)))
            elif kind == "cor":
                corners = [a_corners(qb, g, j) for j in range(4)]
            elif kind == "head":
                ps.append(a_probs(qb, g, i, corners[i]))
            elif kind == "av":
                a_values(qb, g, ps)
            elif kind == "fin":
                finish(jnp.maximum(qb - 1, 0), g)
        o = jnp.concatenate([acc[a] for a in range(5)], axis=0)
        o3 = o[:, 384:512]
        o = jnp.concatenate([o[:, 0:384], o3 + pltpu.roll(o3, 64, 1)], axis=1)
        bs[32 * g:32 * (g + 1), :] = o[8:40].astype(BF16)
        return o[0:8]

    def main(qb, mem):
        retire()
        for g in range(4):
            mem = step(qb, g, mem)

        @pl.when(qb > 0)
        def _():
            out_copy(qb - 1).start()
        return mem

    jax.lax.fori_loop(0, NB, main, m0)

    retire()
    for g in range(4):
        finish(NB - 1, g)
    out_copy(NB - 1).start()
    for qb in range(NB):
        out_copy(qb).wait()


@functools.partial(jax.jit, static_argnames=("B_seg_len",))
def pallas_gated_mix__sliding_block__memory_aug_recurrent_mem_tr__prompt_kernel(
    A_x, A_wqkv, A_wo, B_x, B_mem0, B_Wq, B_Wk, B_Wv, B_Wo, B_seg_len, gate_w,
):
    del B_x
    assert A_x.shape == (1, S, D) and B_Wq.shape == (D, 16, 256) and B_seg_len == 32
    hbm = pl.BlockSpec(memory_space=pl.ANY)
    outT = pl.pallas_call(
        _kernel,
        out_shape=jax.ShapeDtypeStruct((D, S), BF16),
        in_specs=[hbm] * 9,
        out_specs=hbm,
        scratch_shapes=[
            pltpu.VMEM((XC, D, S // XC), BF16),
            pltpu.VMEM((D, 3 * D), BF16),
            pltpu.VMEM((D, D), BF16),
            pltpu.VMEM((3, 2, 16 * D, 128), BF16),
            pltpu.VMEM((16, D, 256), BF16),
            pltpu.VMEM((3 * D + 16, D), BF16),
            pltpu.VMEM((D, D), BF16),
            pltpu.VMEM((S, 512), BF16),
            pltpu.VMEM((NB, D, 128), BF16),
            pltpu.VMEM((4, 256 + S, 128), BF16),
            pltpu.VMEM((4, NB, 96, 128), BF16),
            pltpu.VMEM((NB + 2, 512, 128), BF16),
            pltpu.VMEM((NB, 8, 128), F32),
            pltpu.VMEM((40, 15, 64, 128), U32),
            pltpu.VMEM((8, 32, 128), U32),
            pltpu.VMEM((8, 4, 64, 128), U32),
            pltpu.VMEM((2, 2, 2, 2, D // 2, 128), U32),
            pltpu.VMEM((9, 4, 128, 128), BF16),
            pltpu.VMEM((9, 4, 128, 128), BF16),
            pltpu.VMEM((40, 6, 32, 128), F32),
            pltpu.VMEM((8, 32, 128), F32),
            pltpu.VMEM((8, 40, 128), F32),
            pltpu.VMEM((3, 8, 128), F32),
            pltpu.VMEM((12, 384, 128), F32),
            pltpu.VMEM((D, 128), BF16),
            pltpu.VMEM((D, 128), BF16),
            pltpu.VMEM((128, 512), BF16),
            pltpu.VMEM((512, 128), BF16),
            pltpu.VMEM((NB, D, 128), BF16),
            pltpu.VMEM((64, 128), U32),
            pltpu.VMEM((8, D), BF16),
            pltpu.VMEM((D,), BF16),
            pltpu.SemaphoreType.DMA((XC,)),
            pltpu.SemaphoreType.DMA((5,)),
            pltpu.SemaphoreType.DMA((7,)),
            pltpu.SemaphoreType.DMA((NB,)),
        ],
        compiler_params=pltpu.CompilerParams(vmem_limit_bytes=100 * 1024 * 1024),
    )(jnp.transpose(A_x.reshape(S, D)), A_wqkv, A_wo, B_mem0.reshape(8, D),
      B_Wq.reshape(16 * D, 256), B_Wk.reshape(16 * D, 256), B_Wv.reshape(16 * D, 256),
      jnp.transpose(B_Wo, (0, 2, 1)), gate_w)
    return jnp.transpose(outT).reshape(1, S, D)
```
